```python
import jax
import jax.numpy as jnp

def _softmax(x, axis=-1):
    return jax.nn.softmax(x, axis=axis)
def _gelu(x):
    return jax.nn.gelu(x, approximate=True)
def _silu(x):
    return jax.nn.silu(x)
def _sigmoid(x):
    return jax.nn.sigmoid(x)
def _layernorm(x, axis=-1, eps=1e-5):
    m = jnp.mean(x, axis=axis, keepdims=True)
    v = jnp.var(x, axis=axis, keepdims=True)
    return (x - m) / jnp.sqrt(v + eps)
def _scatter_add(tgt, idx, src, axis=0):
    return tgt.at[idx].add(src)
def _segment_sum(src, seg, n):
    return jax.ops.segment_sum(src, seg, n)
class _Rng:
    def __init__(self, key):
        self._k = key
    def _next(self):
        self._k, sub = jax.random.split(self._k)
        return sub
    def normal(self, shape):
        return jax.random.normal(self._next(), shape, dtype=jnp.bfloat16)
    def randint(self, lo, hi, shape):
        return jax.random.randint(self._next(), shape, lo, hi, dtype=jnp.int32)
    def uniform(self, shape, lo=0.0, hi=1.0):
        return jax.random.uniform(self._next(), shape, jnp.bfloat16, lo, hi)
    def permutation(self, n):
        return jax.random.permutation(self._next(), n)


kernel_name = 'standalone__gqa_softmax__near_ridge'

def setup_inputs():
    _rng = _Rng(jax.random.key(int.from_bytes(__import__("os").urandom(4), "little")))
    _w = (lambda a: (lambda t: t.astype(jnp.bfloat16) if jnp.issubdtype(t.dtype, jnp.floating) else t)(jnp.asarray(a)))
    B, Hq, Hkv, Sq, Sk, D = 16, 32, 32, 848, 512, 192
    return {
        "q": _w((lambda *s: _rng.normal(s) * 0.05)(B, Hq, Sq, D)),
        "k": _w((lambda *s: _rng.normal(s) * 0.05)(B, Hkv, Sk, D)),
        "v": _w((lambda *s: _rng.normal(s) * 0.05)(B, Hkv, Sk, D)),
    }

def reference(q, k, v):
    B, Hq, Sq, D = q.shape
    Hkv = k.shape[1]
    rep = Hq // Hkv
    k = jnp.repeat(k, rep, axis=1)
    v = jnp.repeat(v, rep, axis=1)
    scale = D ** -0.5
    scores = jnp.einsum("bhqd,bhkd->bhqk", q, k) * scale
    p = _softmax(scores, axis=-1)
    return jnp.einsum("bhqk,bhkd->bhqd", p, v)
```

```python
import functools

import jax
import jax.numpy as jnp
from jax import lax
import jax.experimental.pallas as pl
import jax.experimental.pallas.tpu as pltpu

_LOG2E = 1.4426950408889634


def _attn_kernel(q_ref, k_ref, v_ref, o_ref, *, c, hb):
    for h in range(hb):
        qT = q_ref[h]
        kT = k_ref[h]
        vT = v_ref[h]
        sT = lax.dot_general(kT, qT, (((0,), (0,)), ((), ())),
                             preferred_element_type=jnp.float32)
        m = jnp.max(sT, axis=0, keepdims=True)
        p = jnp.exp2((sT - m) * c)
        l = jnp.sum(p, axis=0, keepdims=True)
        oT = jnp.dot(vT, p.astype(jnp.bfloat16), preferred_element_type=jnp.float32)
        o_ref[h] = (oT * (1.0 / l)).astype(o_ref.dtype)


@jax.jit
def pallas_standalone__gqa_softmax__near_ridge_kernel(
    q: jax.Array,
    k: jax.Array,
    v: jax.Array,
):
    B, H, Sq, D = q.shape
    Hkv, Sk = k.shape[1], k.shape[2]
    assert H == Hkv
    hb = 2
    qT = jnp.swapaxes(q, 2, 3).reshape(B * H, D, Sq)
    kT = jnp.swapaxes(k, 2, 3).reshape(B * H, D, Sk)
    vT = jnp.swapaxes(v, 2, 3).reshape(B * H, D, Sk)
    c = float(D ** -0.5 * _LOG2E)
    oT = pl.pallas_call(
        functools.partial(_attn_kernel, c=c, hb=hb),
        grid=(B * H // hb,),
        in_specs=[pl.BlockSpec((hb, D, Sq), lambda i: (i, 0, 0)),
                  pl.BlockSpec((hb, D, Sk), lambda i: (i, 0, 0)),
                  pl.BlockSpec((hb, D, Sk), lambda i: (i, 0, 0))],
        out_specs=pl.BlockSpec((hb, D, Sq), lambda i: (i, 0, 0)),
        out_shape=jax.ShapeDtypeStruct((B * H, D, Sq), q.dtype),
        compiler_params=pltpu.CompilerParams(
            dimension_semantics=("parallel",), vmem_limit_bytes=64 * 1024 * 1024),
    )(qT, kT, vT)
    return jnp.swapaxes(oT.reshape(B, H, D, Sq), 2, 3)
```

```python
import functools

import jax
import jax.numpy as jnp
import jax.experimental.pallas as pl
import jax.experimental.pallas.tpu as pltpu

_LOG2E = 1.4426950408889634
_F32 = jnp.float32
_BF16 = jnp.bfloat16
_U32 = jnp.uint32


def _cat16(a, b):
    cat = jnp.concatenate([pltpu.bitcast(a, _U32), pltpu.bitcast(b, _U32)], 0)
    return pltpu.bitcast(cat, _BF16)


def _prep_k(k_ref, h):
    _, D, Sk = k_ref.shape
    t = D // 3
    n = Sk // 2
    a1, a2 = k_ref[h, 0:t, :n], k_ref[h, 0:t, n:]
    b1, b2 = k_ref[h, t:2 * t, :n], k_ref[h, t:2 * t, n:]
    c1, c2 = k_ref[h, 2 * t:, :n], k_ref[h, 2 * t:, n:]
    db = (b1.astype(_F32) - b2.astype(_F32)).astype(_BF16)
    da = (a2.astype(_F32) - a1.astype(_F32)).astype(_BF16)
    return _cat16(a1, b2).T, _cat16(db, c1).T, _cat16(da, c2).T


def _qk(q_ref, h, s, e, ls):
    t = q_ref.shape[1] // 3
    l0, l1, l2 = ls
    qa, qb, qc = q_ref[h, 0:t, s:e], q_ref[h, t:2 * t, s:e], q_ref[h, 2 * t:, s:e]
    shared = jnp.dot(l0, _cat16(qa, qb), preferred_element_type=_F32)
    s1 = shared + jnp.dot(l1, _cat16(qb, qc), preferred_element_type=_F32)
    s2 = shared + jnp.dot(l2, _cat16(qa, qc), preferred_element_type=_F32)
    return s1, s2


def _softmax(s1, s2, c):
    m = jnp.max(jnp.maximum(s1, s2), axis=0, keepdims=True)
    p1 = jnp.exp2((s1 - m) * c)
    p2 = jnp.exp2((s2 - m) * c)
    l = jnp.sum(p1 + p2, axis=0, keepdims=True)
    return jnp.concatenate([p1, p2], 0).astype(_BF16), l


def _attn_kernel(q_ref, k_ref, v_ref, o_ref, *, c, hb, depth):
    Sq = q_ref.shape[2]
    units = [(h, s, min(s + 128, Sq)) for h in range(hb) for s in range(0, Sq, 128)]
    ls, scores = {}, {}
    for i in range(len(units) + depth):
        if i < len(units):
            h, s, e = units[i]
            if h not in ls:
                ls[h] = _prep_k(k_ref, h)
            scores[i] = _qk(q_ref, h, s, e, ls[h])
        if i >= depth:
            h, s, e = units[i - depth]
            p, l = _softmax(*scores.pop(i - depth), c)
            oT = jnp.dot(v_ref[h], p, preferred_element_type=_F32)
            o_ref[h, :, s:e] = (oT * (1.0 / l)).astype(o_ref.dtype)


@jax.jit
def pallas_standalone__gqa_softmax__near_ridge_kernel(
    q: jax.Array,
    k: jax.Array,
    v: jax.Array,
):
    B, H, Sq, D = q.shape
    Hkv, Sk = k.shape[1], k.shape[2]
    assert H == Hkv
    hb = 8
    qT = jnp.swapaxes(q, 2, 3).reshape(B * H, D, Sq)
    kT = jnp.swapaxes(k, 2, 3).reshape(B * H, D, Sk)
    vT = jnp.swapaxes(v, 2, 3).reshape(B * H, D, Sk)
    c = float(D ** -0.5 * _LOG2E)
    oT = pl.pallas_call(
        functools.partial(_attn_kernel, c=c, hb=hb, depth=3),
        grid=(B * H // hb,),
        in_specs=[pl.BlockSpec((hb, D, Sq), lambda i: (i, 0, 0)),
                  pl.BlockSpec((hb, D, Sk), lambda i: (i, 0, 0)),
                  pl.BlockSpec((hb, D, Sk), lambda i: (i, 0, 0))],
        out_specs=pl.BlockSpec((hb, D, Sq), lambda i: (i, 0, 0)),
        out_shape=jax.ShapeDtypeStruct((B * H, D, Sq), q.dtype),
        compiler_params=pltpu.CompilerParams(
            dimension_semantics=("parallel",),
            vmem_limit_bytes=100 * 1024 * 1024,
            flags={"XLA_TPU_FORCE_LP_LLO_SCHEDULER": True}),
    )(qT, kT, vT)
    return jnp.swapaxes(oT.reshape(B, H, D, Sq), 2, 3)
```

```python
import functools

import jax
import jax.numpy as jnp
from jax import lax
import jax.experimental.pallas as pl
import jax.experimental.pallas.tpu as pltpu

_LOG2E = 1.4426950408889634
_F32 = jnp.float32
_BF16 = jnp.bfloat16
_U32 = jnp.uint32
_LANES = 128


def _dot(a, b, ca, cb):
    return lax.dot_general(a, b, (((ca,), (cb,)), ((), ())), preferred_element_type=_F32)


def _cat16(a, b):
    cat = jnp.concatenate([pltpu.bitcast(a, _U32), pltpu.bitcast(b, _U32)], 0)
    return pltpu.bitcast(cat, _BF16)


def _prep_k(k_ref):
    D, Sk = k_ref.shape
    t, n = D // 3, Sk // 2
    a1, a2 = k_ref[0:t, :n], k_ref[0:t, n:]
    b1, b2 = k_ref[t:2 * t, :n], k_ref[t:2 * t, n:]
    c1, c2 = k_ref[2 * t:, :n], k_ref[2 * t:, n:]
    db = (b1.astype(_F32) - b2.astype(_F32)).astype(_BF16)
    da = (a2.astype(_F32) - a1.astype(_F32)).astype(_BF16)
    d_major = (_cat16(a1, b2), _cat16(db, c1), _cat16(da, c2))
    return d_major, tuple(x.T for x in d_major)


def _scores(q_ref, s, e, keys):
    t = q_ref.shape[0] // 3
    qa, qb, qc = q_ref[0:t, s:e], q_ref[t:2 * t, s:e], q_ref[2 * t:, s:e]
    w0, w1, w2 = _cat16(qa, qb), _cat16(qb, qc), _cat16(qa, qc)
    if e - s < _LANES:
        k0, k1, k2 = keys[0]
        shared = _dot(w0, k0, 0, 0)
        return shared + _dot(w1, k1, 0, 0), shared + _dot(w2, k2, 0, 0)
    k0, k1, k2 = keys[1]
    shared = _dot(k0, w0, 1, 0)
    return shared + _dot(k1, w1, 1, 0), shared + _dot(k2, w2, 1, 0)


def _softmax_pv(v_ref, o_ref, s, e, s1, s2, c):
    w = e - s
    if w < _LANES:
        m = jnp.max(jnp.maximum(s1, s2), axis=1, keepdims=True)
        p1 = jnp.exp2((s1 - m) * c)
        p2 = jnp.exp2((s2 - m) * c)
        r = 1.0 / jnp.sum(p1 + p2, axis=1, keepdims=True)
        p = jnp.concatenate([p1 * r, p2 * r], 1).astype(_BF16)
        lo = _dot(p, v_ref[:_LANES, :], 1, 1)
        o_ref[:_LANES, s:e] = lo.T.astype(o_ref.dtype)
        o_ref[_LANES:, s:e] = _dot(v_ref[_LANES:, :], p, 1, 1).astype(o_ref.dtype)
        return
    n = s1.shape[0]
    m = jnp.max(jnp.maximum(s1, s2), axis=0, keepdims=True)
    m = jnp.broadcast_to(m, (8, w))
    p1 = jnp.exp2((s1.reshape(n // 8, 8, w) - m[None]) * c)
    l1 = jnp.sum(p1, axis=0)
    m = jnp.maximum(m, jnp.minimum(m, l1))
    p2 = jnp.exp2((s2.reshape(n // 8, 8, w) - m[None]) * c)
    l = jnp.sum(l1 + jnp.sum(p2, axis=0), axis=0, keepdims=True)
    p = jnp.concatenate([p1.reshape(n, w), p2.reshape(n, w)], 0).astype(_BF16)
    o_ref[:, s:e] = (_dot(v_ref[...], p, 1, 0) * (1.0 / l)).astype(o_ref.dtype)


def _attn_kernel(q_ref, k_ref, v_ref, o_ref, *, c, depth):
    heads, _, Sq = q_ref.shape
    cols = [(s, min(s + _LANES, Sq)) for s in range(0, Sq, _LANES)]
    cols.insert(0, cols.pop())
    units = [(h, s, e) for h in range(heads) for s, e in cols]
    keys, scores = {}, {}
    for i in range(len(units) + depth):
        if i < len(units):
            h, s, e = units[i]
            if h not in keys:
                keys[h] = _prep_k(k_ref.at[h])
            scores[i] = _scores(q_ref.at[h], s, e, keys[h])
        if i >= depth:
            h, s, e = units[i - depth]
            _softmax_pv(v_ref.at[h], o_ref.at[h], s, e, *scores.pop(i - depth), c)


@jax.jit
def pallas_standalone__gqa_softmax__near_ridge_kernel(
    q: jax.Array,
    k: jax.Array,
    v: jax.Array,
):
    B, H, Sq, D = q.shape
    Hkv, Sk = k.shape[1], k.shape[2]
    assert H == Hkv and D == 192
    hb = 8
    qT = jnp.swapaxes(q, 2, 3).reshape(B * H, D, Sq)
    kT = jnp.swapaxes(k, 2, 3).reshape(B * H, D, Sk)
    vT = jnp.swapaxes(v, 2, 3).reshape(B * H, D, Sk)
    c = float(D ** -0.5 * _LOG2E)
    oT = pl.pallas_call(
        functools.partial(_attn_kernel, c=c, depth=3),
        grid=(B * H // hb,),
        in_specs=[pl.BlockSpec((hb, D, Sq), lambda i: (i, 0, 0)),
                  pl.BlockSpec((hb, D, Sk), lambda i: (i, 0, 0)),
                  pl.BlockSpec((hb, D, Sk), lambda i: (i, 0, 0))],
        out_specs=pl.BlockSpec((hb, D, Sq), lambda i: (i, 0, 0)),
        out_shape=jax.ShapeDtypeStruct((B * H, D, Sq), q.dtype),
        compiler_params=pltpu.CompilerParams(
            dimension_semantics=("parallel",),
            vmem_limit_bytes=100 * 1024 * 1024,
            flags={"XLA_TPU_FORCE_LP_LLO_SCHEDULER": True}),
    )(qT, kT, vT)
    return jnp.swapaxes(oT.reshape(B, H, D, Sq), 2, 3)
```

```python
import functools

import jax
import jax.numpy as jnp
from jax import lax
import jax.experimental.pallas as pl
import jax.experimental.pallas.tpu as pltpu

_LOG2E = 1.4426950408889634
_F32 = jnp.float32
_BF16 = jnp.bfloat16
_LANES = 128
_DEPTH = 3
_BIG = 18
_SMALL = 2


def _dot(a, b, ca, cb):
    return lax.dot_general(a, b, (((ca,), (cb,)), ((), ())), preferred_element_type=_F32)


def _cat16(a, b):
    cat = jnp.concatenate([pltpu.bitcast(a, jnp.uint32), pltpu.bitcast(b, jnp.uint32)], 0)
    return pltpu.bitcast(cat, _BF16)


def _after(m, x):
    m, x = pltpu.bitcast(m, jnp.int32), pltpu.bitcast(x, jnp.int32)
    return pltpu.bitcast(jnp.maximum(m, jnp.minimum(m, x)), _F32)


def _prep_k(k_ref):
    D, Sk = k_ref.shape
    t, n = D // 3, Sk // 2
    a1, a2 = k_ref[0:t, :n], k_ref[0:t, n:]
    b1, b2 = k_ref[t:2 * t, :n], k_ref[t:2 * t, n:]
    c1, c2 = k_ref[2 * t:, :n], k_ref[2 * t:, n:]
    db = (b1.astype(_F32) - b2.astype(_F32)).astype(_BF16)
    da = (a2.astype(_F32) - a1.astype(_F32)).astype(_BF16)
    d_major = (_cat16(a1, b2), _cat16(db, c1), _cat16(da, c2))
    return d_major, tuple(x.T for x in d_major)


def _scores(q_ref, s, e, keys):
    t = q_ref.shape[0] // 3
    qa, qb, qc = q_ref[0:t, s:e], q_ref[t:2 * t, s:e], q_ref[2 * t:, s:e]
    w0, w1, w2 = _cat16(qa, qb), _cat16(qb, qc), _cat16(qa, qc)
    if e - s < _LANES:
        k0, k1, k2 = keys[0]
        shared, r2, r1 = _dot(w0, k0, 0, 0), _dot(w2, k2, 0, 0), _dot(w1, k1, 0, 0)
    else:
        k0, k1, k2 = keys[1]
        shared, r2, r1 = _dot(k0, w0, 1, 0), _dot(k2, w2, 1, 0), _dot(k1, w1, 1, 0)
    return shared + r1, shared + r2


def _softmax_pv_ragged(v_ref, o_ref, s, e, s1, s2, c):
    m = jnp.max(jnp.maximum(s1, s2), axis=1, keepdims=True)
    p1 = jnp.exp2((s1 - m) * c)
    l1 = p1[:, :_LANES] + p1[:, _LANES:]
    m = _after(jnp.broadcast_to(m, l1.shape), l1)
    p2 = jnp.exp2((s2 - jnp.concatenate([m, m], 1)) * c)
    l = jnp.sum(l1 + p2[:, :_LANES] + p2[:, _LANES:], axis=1, keepdims=True)
    r = 1.0 / l
    p = jnp.concatenate([p1 * r, p2 * r], 1).astype(_BF16)
    o_ref[:_LANES, s:e] = _dot(p, v_ref[:_LANES, :], 1, 1).T.astype(o_ref.dtype)
    o_ref[_LANES:, s:e] = _dot(v_ref[_LANES:, :], p, 1, 1).astype(o_ref.dtype)


def _softmax_pv(v_ref, o_ref, s, e, s1, s2, c, prev):
    w = e - s
    m = jnp.max(jnp.maximum(s1, s2), axis=0, keepdims=True)
    m = jnp.broadcast_to(m, (8, w))
    if prev is not None:
        m = _after(m, prev)
    sc = jnp.concatenate([s1, s2], 0)
    n = sc.shape[0]
    p = jnp.exp2((sc.reshape(n // 8, 8, w) - m[None]) * c)
    part = jnp.sum(p, axis=0)
    l = jnp.sum(part, axis=0, keepdims=True)
    o = _dot(v_ref[...], p.reshape(n, w).astype(_BF16), 1, 0)
    o_ref[:, s:e] = (o * (1.0 / l)).astype(o_ref.dtype)
    return part


def _attend(q_ref, k_ref, v_ref, o_ref, c):
    heads, _, Sq = q_ref.shape
    cols = [(s, min(s + _LANES, Sq)) for s in range(0, Sq, _LANES)]
    cols.insert(0, cols.pop())
    tiles = [(h, s, e) for h in range(heads) for s, e in cols]
    keys, scores, prev = {}, {}, None
    for i in range(len(tiles) + _DEPTH):
        if i < len(tiles):
            h, s, e = tiles[i]
            if h not in keys:
                keys[h] = _prep_k(k_ref.at[h])
            scores[i] = _scores(q_ref.at[h], s, e, keys[h])
        if i >= _DEPTH:
            h, s, e = tiles[i - _DEPTH]
            s1, s2 = scores.pop(i - _DEPTH)
            if e - s < _LANES:
                _softmax_pv_ragged(v_ref.at[h], o_ref.at[h], s, e, s1, s2, c)
            else:
                prev = _softmax_pv(v_ref.at[h], o_ref.at[h], s, e, s1, s2, c, prev)


def _attn_kernel(q_hbm, k_hbm, v_hbm, o_hbm, q_big, k_big, v_big, o_big,
                 q_small, k_small, v_small, o_small, sem_big, sem_small, *, c):
    n_big = q_hbm.shape[0] // _BIG - 1
    n_up = _BIG // _SMALL
    n_small = q_small.shape[0] // _SMALL

    def big_in(g, slot, off=0, cnt=_BIG):
        src, dst = pl.ds((g + 1) * _BIG + off, cnt), pl.ds(off, cnt)
        return [pltpu.make_async_copy(a.at[src], b.at[slot, dst], sem_big.at[4 * slot + i])
                for i, (a, b) in enumerate(((k_hbm, k_big), (q_hbm, q_big), (v_hbm, v_big)))]

    def big_out(g, slot):
        dst = o_hbm.at[pl.ds((g + 1) * _BIG, _BIG)]
        return pltpu.make_async_copy(o_big.at[slot], dst, sem_big.at[4 * slot + 3])

    def small_heads(j):
        return pl.ds(j * _SMALL + jnp.where(j >= n_up, n_big * _BIG, 0), _SMALL)

    def small_in(j):
        src, dst = small_heads(j), pl.ds(j * _SMALL, _SMALL)
        return [pltpu.make_async_copy(a.at[src], b.at[dst], sem_small.at[4 * j + i])
                for i, (a, b) in enumerate(((k_hbm, k_small), (q_hbm, q_small), (v_hbm, v_small)))]

    def small_out(j):
        src = o_small.at[pl.ds(j * _SMALL, _SMALL)]
        return pltpu.make_async_copy(src, o_hbm.at[small_heads(j)], sem_small.at[4 * j + 3])

    def small_attend(j):
        heads = pl.ds(j * _SMALL, _SMALL)
        _attend(q_small.at[heads], k_small.at[heads], v_small.at[heads], o_small.at[heads], c)

    up_out = pltpu.make_async_copy(
        o_small.at[pl.ds(0, _BIG)], o_hbm.at[pl.ds(0, _BIG)], sem_small.at[3])

    def start(copies):
        for copy in copies:
            copy.start()

    def wait(copies):
        for copy in copies:
            copy.wait()

    def ramp_up(j, carry):
        wait(small_in(j))
        for t in range(2):
            i = 2 * j + 1 + t

            @pl.when(i < n_up)
            def _():
                start(small_in(i))

            @pl.when(jnp.logical_and(i >= n_up, i < 2 * n_up))
            def _():
                start(big_in(0, 0, (i - n_up) * _SMALL, _SMALL))

        small_attend(j)
        return carry

    def main(g, carry):
        slot = g % 2
        wait(big_in(g, slot))

        @pl.when(g + 1 < n_big)
        def _():
            start(big_in(g + 1, 1 - slot))

        @pl.when(g + 1 == n_big)
        def _():
            for j in range(n_up, n_small):
                start(small_in(j))

        @pl.when(g == 0)
        def _():
            up_out.start()

        @pl.when(g >= 2)
        def _():
            big_out(g - 2, slot).wait()

        _attend(q_big.at[slot], k_big.at[slot], v_big.at[slot], o_big.at[slot], c)
        big_out(g, slot).start()
        return carry

    def ramp_down(j, carry):
        wait(small_in(j))
        small_attend(j)
        small_out(j).start()
        return carry

    start(small_in(0))
    lax.fori_loop(0, n_up, ramp_up, 0)
    lax.fori_loop(0, n_big, main, 0)
    lax.fori_loop(n_up, n_small, ramp_down, 0)
    up_out.wait()
    wait([big_out(g, g % 2) for g in (n_big - 2, n_big - 1)])
    wait([small_out(j) for j in range(n_up, n_small)])


@jax.jit
def pallas_standalone__gqa_softmax__near_ridge_kernel(
    q: jax.Array,
    k: jax.Array,
    v: jax.Array,
):
    B, H, Sq, D = q.shape
    Sk = k.shape[2]
    N = B * H
    assert k.shape[1] == H and D == 192 and Sk == 512 and Sq % _LANES
    assert N % _SMALL == 0 and _BIG % _SMALL == 0 and N >= 3 * _BIG
    n_small = _BIG + N % _BIG
    qT = jnp.swapaxes(q, 2, 3).reshape(N, D, Sq)
    kT = jnp.swapaxes(k, 2, 3).reshape(N, D, Sk)
    vT = jnp.swapaxes(v, 2, 3).reshape(N, D, Sk)
    in_hbm = pl.BlockSpec(memory_space=pl.ANY)
    oT = pl.pallas_call(
        functools.partial(_attn_kernel, c=float(D ** -0.5 * _LOG2E)),
        in_specs=[in_hbm] * 3,
        out_specs=in_hbm,
        out_shape=jax.ShapeDtypeStruct((N, D, Sq), q.dtype),
        scratch_shapes=(
            [pltpu.VMEM((2, _BIG, D, s), _BF16) for s in (Sq, Sk, Sk, Sq)]
            + [pltpu.VMEM((n_small, D, s), _BF16) for s in (Sq, Sk, Sk, Sq)]
            + [pltpu.SemaphoreType.DMA((8,)),
               pltpu.SemaphoreType.DMA((4 * n_small // _SMALL,))]),
        compiler_params=pltpu.CompilerParams(
            vmem_limit_bytes=100 * 1024 * 1024,
            flags={"XLA_TPU_FORCE_LP_LLO_SCHEDULER": True}),
    )(qT, kT, vT)
    return jnp.swapaxes(oT.reshape(B, H, D, Sq), 2, 3)
```

```python
import functools

import jax
import jax.numpy as jnp
from jax import lax
import jax.experimental.pallas as pl
import jax.experimental.pallas.tpu as pltpu

_LOG2E = 1.4426950408889634
_F32 = jnp.float32
_BF16 = jnp.bfloat16
_LANES = 128
_DEPTH = 3
_BIG = 18
_SMALL = 2


def _dot(a, b, ca, cb):
    return lax.dot_general(a, b, (((ca,), (cb,)), ((), ())), preferred_element_type=_F32)


def _cat16(a, b):
    cat = jnp.concatenate([pltpu.bitcast(a, jnp.uint32), pltpu.bitcast(b, jnp.uint32)], 0)
    return pltpu.bitcast(cat, _BF16)


def _after(m, x):
    m, x = pltpu.bitcast(m, jnp.int32), pltpu.bitcast(x, jnp.int32)
    return pltpu.bitcast(jnp.maximum(m, jnp.minimum(m, x)), _F32)


def _prep_k(k_ref):
    D, Sk = k_ref.shape
    t, n = D // 3, Sk // 2
    a1, a2 = k_ref[0:t, :n], k_ref[0:t, n:]
    b1, b2 = k_ref[t:2 * t, :n], k_ref[t:2 * t, n:]
    c1, c2 = k_ref[2 * t:, :n], k_ref[2 * t:, n:]
    db = (b1.astype(_F32) - b2.astype(_F32)).astype(_BF16)
    da = (a2.astype(_F32) - a1.astype(_F32)).astype(_BF16)
    d_major = (_cat16(a1, b2), _cat16(db, c1), _cat16(da, c2))
    return d_major, tuple(x.T for x in d_major)


def _scores(q_ref, s, e, keys):
    t = q_ref.shape[0] // 3
    qa, qb, qc = q_ref[0:t, s:e], q_ref[t:2 * t, s:e], q_ref[2 * t:, s:e]
    w0, w1, w2 = _cat16(qa, qb), _cat16(qb, qc), _cat16(qa, qc)
    if e - s < _LANES:
        k0, k1, k2 = keys[0]
        shared, r2, r1 = _dot(w0, k0, 0, 0), _dot(w2, k2, 0, 0), _dot(w1, k1, 0, 0)
    else:
        k0, k1, k2 = keys[1]
        shared, r2, r1 = _dot(k0, w0, 1, 0), _dot(k2, w2, 1, 0), _dot(k1, w1, 1, 0)
    return shared + r1, shared + r2


def _softmax_pv_ragged(v_ref, o_ref, s, e, s1, s2, c):
    m = jnp.max(jnp.maximum(s1, s2), axis=1, keepdims=True)
    p1 = jnp.exp2((s1 - m) * c)
    l1 = p1[:, :_LANES] + p1[:, _LANES:]
    m = _after(jnp.broadcast_to(m, l1.shape), l1)
    p2 = jnp.exp2((s2 - jnp.concatenate([m, m], 1)) * c)
    l = jnp.sum(l1 + p2[:, :_LANES] + p2[:, _LANES:], axis=1, keepdims=True)
    r = 1.0 / l
    p = jnp.concatenate([p1 * r, p2 * r], 1).astype(_BF16)
    o_ref[:_LANES, s:e] = _dot(p, v_ref[:_LANES, :], 1, 1).T.astype(o_ref.dtype)
    o_ref[_LANES:, s:e] = _dot(v_ref[_LANES:, :], p, 1, 1).astype(o_ref.dtype)


def _softmax_pv(v_ref, o_ref, s, e, s1, s2, c, prev):
    w = e - s
    m = jnp.max(jnp.maximum(s1, s2), axis=0, keepdims=True)
    m = jnp.broadcast_to(m, (8, w))
    if prev is not None:
        m = _after(m, prev)
    sc = jnp.concatenate([s1, s2], 0)
    n = sc.shape[0]
    p = jnp.exp2((sc.reshape(n // 8, 8, w) - m[None]) * c)
    part = jnp.sum(p, axis=0)
    l = jnp.sum(part, axis=0, keepdims=True)
    o = _dot(v_ref[...], p.reshape(n, w).astype(_BF16), 1, 0)
    o_ref[:, s:e] = (o * (1.0 / l)).astype(o_ref.dtype)
    return part


def _attend(q_ref, k_ref, v_ref, o_ref, c):
    heads, _, Sq = q_ref.shape
    cols = [(s, min(s + _LANES, Sq)) for s in range(0, Sq, _LANES)]
    cols.insert(0, cols.pop())
    tiles = [(h, s, e) for h in range(heads) for s, e in cols]
    keys, scores, prev = {}, {}, None
    for i in range(len(tiles) + _DEPTH):
        if i < len(tiles):
            h, s, e = tiles[i]
            if h not in keys:
                keys[h] = _prep_k(k_ref.at[h])
            scores[i] = _scores(q_ref.at[h], s, e, keys[h])
        if i >= _DEPTH:
            h, s, e = tiles[i - _DEPTH]
            s1, s2 = scores.pop(i - _DEPTH)
            if e - s < _LANES:
                _softmax_pv_ragged(v_ref.at[h], o_ref.at[h], s, e, s1, s2, c)
            else:
                prev = _softmax_pv(v_ref.at[h], o_ref.at[h], s, e, s1, s2, c, prev)


def _attn_kernel(q_hbm, k_hbm, v_hbm, o_hbm, q_buf, k_buf, v_buf, o_buf, in_sem, out_sem, *, c):
    n_heads = q_hbm.shape[0]
    n_groups = n_heads // _BIG
    n_up = _BIG // _SMALL
    n_down = n_heads % _BIG // _SMALL

    def loads(head, pos, count, sem):
        src, dst = pl.ds(head, count), pl.ds(pos, count)
        return [pltpu.make_async_copy(a.at[src], b.at[dst], in_sem.at[3 * sem + i])
                for i, (a, b) in enumerate(((k_hbm, k_buf), (q_hbm, q_buf), (v_hbm, v_buf)))]

    def store(head, pos, count, sem):
        return pltpu.make_async_copy(
            o_buf.at[pl.ds(pos, count)], o_hbm.at[pl.ds(head, count)], out_sem.at[sem])

    def start(copies):
        for copy in copies:
            copy.start()

    def wait(copies):
        for copy in copies:
            copy.wait()

    def attend(pos, count):
        heads = pl.ds(pos, count)
        _attend(q_buf.at[heads], k_buf.at[heads], v_buf.at[heads], o_buf.at[heads], c)

    def piece(i):
        return loads(i * _SMALL, i * _SMALL, _SMALL, jnp.where(i < n_up, 2 + i, 1))

    def group_in(g):
        return loads(jnp.minimum(g * _BIG, n_heads - _BIG), (g & 1) * _BIG, _BIG, g & 1)

    def group_out(g):
        return store(g * _BIG, (g & 1) * _BIG, _BIG, g & 1)

    def down_pos(j):
        return (n_groups % 2 + 1) * _BIG - (n_down - j) * _SMALL

    def down_out(j):
        return store(n_groups * _BIG + j * _SMALL, down_pos(j), _SMALL, 2 + j)

    def ramp_up(j, carry):
        wait(piece(j))
        start(piece(2 * j + 1))

        @pl.when(j + 1 < n_up)
        def _():
            start(piece(2 * j + 2))

        attend(j * _SMALL, _SMALL)
        return carry

    def main(g, carry):
        wait(group_in(g))
        start(group_in(g + 1))
        group_out(g - 1).start()

        @pl.when(g >= 2)
        def _():
            group_out(g - 2).wait()

        attend((g & 1) * _BIG, _BIG)
        return carry

    def ramp_down(j, carry):
        attend(down_pos(j), _SMALL)
        down_out(j).start()
        return carry

    start(piece(0))
    lax.fori_loop(0, n_up, ramp_up, 0)
    lax.fori_loop(1, n_groups, main, 0)
    group_out(n_groups - 1).start()
    group_out(n_groups - 2).wait()
    wait(group_in(n_groups))
    lax.fori_loop(0, n_down, ramp_down, 0)
    group_out(n_groups - 1).wait()
    wait([down_out(j) for j in range(n_down)])


@jax.jit
def pallas_standalone__gqa_softmax__near_ridge_kernel(
    q: jax.Array,
    k: jax.Array,
    v: jax.Array,
):
    B, H, Sq, D = q.shape
    Sk = k.shape[2]
    N = B * H
    assert k.shape[1] == H and D == 192 and Sk == 512 and Sq % _LANES
    assert N % _SMALL == 0 and _BIG % _SMALL == 0 and N >= 3 * _BIG
    qT = jnp.swapaxes(q, 2, 3).reshape(N, D, Sq)
    kT = jnp.swapaxes(k, 2, 3).reshape(N, D, Sk)
    vT = jnp.swapaxes(v, 2, 3).reshape(N, D, Sk)
    in_hbm = pl.BlockSpec(memory_space=pl.ANY)
    oT = pl.pallas_call(
        functools.partial(_attn_kernel, c=float(D ** -0.5 * _LOG2E)),
        in_specs=[in_hbm] * 3,
        out_specs=in_hbm,
        out_shape=jax.ShapeDtypeStruct((N, D, Sq), q.dtype),
        scratch_shapes=(
            [pltpu.VMEM((2 * _BIG, D, s), _BF16) for s in (Sq, Sk, Sk, Sq)]
            + [pltpu.SemaphoreType.DMA((3 * (2 + _BIG // _SMALL),)),
               pltpu.SemaphoreType.DMA((2 + _BIG // _SMALL,))]),
        compiler_params=pltpu.CompilerParams(
            vmem_limit_bytes=100 * 1024 * 1024,
            disable_bounds_checks=True,
            flags={"XLA_TPU_FORCE_LP_LLO_SCHEDULER": True}),
    )(qT, kT, vT)
    return jnp.swapaxes(oT.reshape(B, H, D, Sq), 2, 3)
```
